```python
import os as _os
_os.environ.setdefault("JAX_PLATFORMS", "cpu")
import jax
import jax.numpy as jnp

def _softmax(x, axis=-1):
    return jax.nn.softmax(x, axis=axis)
def _gelu(x):
    return jax.nn.gelu(x, approximate=True)
def _silu(x):
    return jax.nn.silu(x)
def _sigmoid(x):
    return jax.nn.sigmoid(x)
def _layernorm(x, axis=-1, eps=1e-5):
    m = jnp.mean(x, axis=axis, keepdims=True)
    v = jnp.var(x, axis=axis, keepdims=True)
    return (x - m) / jnp.sqrt(v + eps)
def _scatter_add(tgt, idx, src, axis=0):
    return tgt.at[idx].add(src)
def _segment_sum(src, seg, n):
    return jax.ops.segment_sum(src, seg, n)
class _Rng:
    def __init__(self, key):
        self._k = key
    def _next(self):
        self._k, sub = jax.random.split(self._k)
        return sub
    def normal(self, shape):
        return jax.random.normal(self._next(), shape, dtype=jnp.bfloat16)
    def randint(self, lo, hi, shape):
        return jax.random.randint(self._next(), shape, lo, hi, dtype=jnp.int32)
    def uniform(self, shape, lo=0.0, hi=1.0):
        return jax.random.uniform(self._next(), shape, jnp.bfloat16, lo, hi)
    def permutation(self, n):
        return jax.random.permutation(self._next(), n)


kernel_name = 'parallel_sum__mha_block__dense_activation_mish__prompt'

def setup_inputs():
    _rng = _Rng(jax.random.key(int.from_bytes(__import__("os").urandom(4), "little")))
    _w = (lambda a: (lambda t: t.astype(jnp.bfloat16) if jnp.issubdtype(t.dtype, jnp.floating) else t)(jnp.asarray(a)))
    def _A_setup():
        B, S, D, H = 1, 2048, 512, 32
        return {
            "x": _w((lambda *s: _rng.normal(s) * 0.05)(B, S, D)),
            "wqkv": _w((lambda *s: _rng.normal(s) * 0.05)(D, 3 * D)),
            "wo": _w((lambda *s: _rng.normal(s) * 0.05)(D, D)),
        }
    _A_in = _A_setup()

    def _B_setup():
        B, S, D, F = 1, 2048, 512, 1792
        return {
            "x": _w((lambda *s: _rng.normal(s) * 0.05)(B, S, D)),
            "w1": _w((lambda *s: _rng.normal(s) * 1.6)(D, F) * (D ** -0.5)),
            "b1": _w((lambda *s: _rng.normal(s) * 0.05)(F)),
            "w2": _w((lambda *s: _rng.normal(s) * 0.05)(F, D) * (F ** -0.5)),
        }
    _B_in = _B_setup()

    return {
        "A_x": _A_in["x"],
        "A_wqkv": _A_in["wqkv"],
        "A_wo": _A_in["wo"],
        "B_x": _B_in["x"],
        "B_w1": _B_in["w1"],
        "B_b1": _B_in["b1"],
        "B_w2": _B_in["w2"],
    }

def reference(A_x, A_wqkv, A_wo, B_x, B_w1, B_b1, B_w2):
    def _A_ref(x, wqkv, wo):
        B, S, D = x.shape
        H = 32
        Dh = D // H
        qkv = (lambda x, *d: x.transpose(*d))((x @ wqkv).reshape(B, S, 3, H, Dh), 2, 0, 3, 1, 4)
        q, k, v = qkv[0], qkv[1], qkv[2]
        scores = jnp.einsum("bhqd,bhkd->bhqk", q, k) * (Dh ** -0.5)
        p = _softmax(scores, axis=-1)
        o = jnp.einsum("bhqk,bhkd->bhqd", p, v)
        return (lambda x, *d: x.transpose(*d))(o, 0, 2, 1, 3).reshape(B, S, D) @ wo

    def _B_ref(x, w1, b1, w2):
        h = jnp.einsum("bsd,df->bsf", x, w1) + b1
        sp = jnp.log1p(jnp.exp(-jnp.abs(h))) + jnp.where(h > 0, h, jnp.zeros_like(h))
        act = h * jnp.tanh(sp)
        return jnp.einsum("bsf,fd->bsd", act, w2)

    x = A_x
    xn = _layernorm(x, axis=-1)
    return x + _A_ref(xn, A_wqkv, A_wo) + _B_ref(xn, B_w1, B_b1, B_w2)
```

```python
import jax
import jax.numpy as jnp
import numpy as np
from jax import lax
import jax.experimental.pallas as pl
import jax.experimental.pallas.tpu as pltpu

F32, BF16, I32 = jnp.float32, jnp.bfloat16, jnp.int32
S, D, H, DH, F = 2048, 512, 32, 16, 1792
BQ = 512
NB = S // BQ
CK = 128
NC = S // CK
G = 2
HP = H // G
LAG = 9
LOG2E = 1.4426950408889634
NT = (((1,), (1,)), ((), ()))
NN = (((1,), (0,)), ((), ()))
ORDER = (1, 3, 2, 4, 0, 5, 6)
DOWN_ORDER = (3, 1, 2, 5, 0, 4, 6)
FFN_COLS = ((0, 256), (256, 512), (512, 768), (768, 896))


def _dot(a, b, dims=NN):
    return lax.dot_general(a, b, dims, preferred_element_type=F32)


def _pk(x):
    return pltpu.bitcast(x.astype(BF16), I32)


def _unpk(x):
    return pltpu.bitcast(x, BF16)


def _after(x, zero):
    return pltpu.bitcast(pltpu.bitcast(x, I32) & zero, F32)


def _mish(h):
    e = jnp.exp2(jnp.minimum(h, 20.0) * LOG2E)
    n = e * (e + 2.0)
    return h * (n * pltpu.reciprocal(n + 2.0, approx=True))


def _pack2(hi, lo):
    lo = lax.shift_right_logical(pltpu.bitcast(lo.astype(BF16).astype(F32), I32), 16)
    hi = pltpu.bitcast(hi, I32)
    mag = jnp.maximum((hi & 0x7FFFFFFF) - lo + 0x8000, 0) & ~0xFFFF
    return (hi & ~0x7FFFFFFF) | mag | lo


def _vpu_scores(kw, lanes, q_rows):
    s = None
    for d in range(DH):
        w = jnp.take_along_axis(kw, lanes[d], axis=1, mode="promise_in_bounds")
        k = jnp.concatenate([pltpu.bitcast(w, F32), pltpu.bitcast(w << 16, F32)], axis=0)
        t = jnp.concatenate([k] * (BQ // 128), axis=1) * jnp.concatenate([q_rows[d]] * 2, axis=0)
        s = t if s is None else s + t
    return s


def _add_rows(acc, p):
    for r in range(0, p.shape[0], 8):
        acc = p[r:r + 8] if acc is None else acc + p[r:r + 8]
    return acc


def _quads(x):
    m, n = x.shape[0] // 2, x.shape[1] // 2
    return x[:m, :n], x[:m, n:], x[m:, :n], x[m:, n:]


def _join(c11, c12, c21, c22):
    return jnp.concatenate(
        [jnp.concatenate([c11, c12], axis=1), jnp.concatenate([c21, c22], axis=1)], axis=0)


def _lhs7(a11, a12, a21, a22):
    return a11 + a22, a21 + a22, a11, a22, a11 + a12, a21 - a11, a12 - a22


def _rhs7(b11, b12, b21, b22):
    return b11 + b22, b11, b12 - b22, b21 - b11, b22, b11 + b12, b21 + b22


def _out4(m):
    return (((m[3] - m[4]) + m[0]) + m[6], m[2] + m[4],
            m[1] + m[3], ((m[2] - m[1]) + m[0]) + m[5])


def _ds(i, n):
    return pl.ds(pl.multiple_of(i * n, n), n)


def _kernel(x_hbm, wqkv_hbm, wo_hbm, w1_hbm, b1_ref, w2_hbm, o_hbm,
            x_v, wqkv_v, w1_v, w2_v, o_v, wt_s, b1_s, xs_s, kc_s,
            k_s, kw_s, qt_s, vt_s, ot_s, l_s, sems):
    def x_blk(i):
        return x_v.at[_ds(i, BQ)]

    cp_x = [pltpu.make_async_copy(x_hbm.at[pl.ds(i * BQ, BQ)], x_blk(i), sems.at[i])
            for i in range(NB)]
    cp_x.append(pltpu.make_async_copy(wo_hbm, x_blk(NB), sems.at[NB]))
    cp_wq, cp_wk, cp_wv = [
        pltpu.make_async_copy(wqkv_hbm.at[:, pl.ds(i * D, D)], wqkv_v.at[i], sems.at[5 + i])
        for i in range(3)]
    cp_w1 = pltpu.make_async_copy(w1_hbm, w1_v, sems.at[8])
    cp_w2 = pltpu.make_async_copy(w2_hbm, w2_v, sems.at[9])

    def cp_o(j):
        return pltpu.make_async_copy(o_v.at[j], o_hbm.at[_ds(j, BQ)], sems.at[10 + j])

    def layernorm(i, r0=0, n=BQ // 2, after=None):
        quads = []
        for half in range(2):
            rows = pl.ds(pl.multiple_of(i * BQ + half * (BQ // 2) + r0, 16), n)
            x = x_v[rows, :].astype(F32)
            if after is not None:
                first = x[:, :128] + jnp.concatenate([after] * (n // 8), axis=0)
                x = jnp.concatenate([first, x[:, 128:]], axis=1)
            xc = x - jnp.mean(x, axis=-1, keepdims=True)
            xn = xc * lax.rsqrt(jnp.mean(xc * xc, axis=-1, keepdims=True) + 1e-5)
            quads += [xn[:, :D // 2], xn[:, D // 2:]]

        def store():
            for m, a in enumerate(_lhs7(*quads)):
                xs_s[i, m, r0 // 2:(r0 + n) // 2, :] = _pk(a)
        return store

    def project_k(i):
        w7 = _rhs7(*_quads(wqkv_v[1].astype(F32)))
        k = _join(*_out4({n: _dot(_unpk(xs_s[i, n]), w7[n].astype(BF16)) for n in ORDER}))
        kc_s[:BQ // 2] = _pk(k)
        kc_s[BQ // 2:] = jnp.concatenate(
            [_pack2(k[e - 16:e - 8], k[e - 8:e]) for e in range(CK, BQ + 1, CK)], axis=0)

    def transpose_operands(m, w):
        b11, b21, b12, b22 = _quads(wqkv_v[w].T.astype(F32))
        for n, b in enumerate(_rhs7(b11, b12, b21, b22)):
            wt_s[m, n] = _pk(b)

    cp_x[0].start()
    cp_wk.start()
    b1_s[...] = jnp.broadcast_to(b1_ref[...].astype(F32).reshape(1, F), (8, F))
    cp_x[0].wait()
    cp_wv.start()
    cp_wq.start()
    layernorm(0)()
    cp_wk.wait()
    for cp in cp_x[1:]:
        cp.start()
    project_k(0)
    cp_wv.wait()
    transpose_operands(0, 2)
    cp_wq.wait()
    transpose_operands(1, 0)

    def project(i, vmax):
        pltpu.make_async_copy(x_blk(i + 1), x_blk(i + 1), sems.at[i + 1]).wait()
        zero = jnp.full((8, 128), i // NB, I32)
        for h in range(H):
            for e in range(G):
                if e != h % G:
                    qt_s[i * G + h % G, h // G, e * 8:e * 8 + 8, :] = jnp.zeros((8, BQ), I32)
        pieces = (32,) * 6 + (16,) * 4
        stores = {}
        for m in range(2):
            ms = {}
            for t, n in enumerate(ORDER, 7 * m):
                ms[n] = _dot(_unpk(wt_s[m, n]), _unpk(xs_s[i, n]), NT)
                if t < len(pieces):
                    stores[t + 3] = layernorm(
                        i + 1, sum(pieces[:t]), pieces[t], _after(ms[n][:8, :128], zero))
                if t in stores:
                    stores.pop(t)()
                for h in range(HP):
                    if t == h * 13 // HP:
                        g, r = divmod(h * G * DH, 128)
                        w = kc_s[:, g * 128:(g + 1) * 128]
                        w = pltpu.roll(w, 128 - r, 1) if r else w
                        k_s[h, _ds(i, BQ // 2), :] = w[:BQ // 2]
                        kw_s[h, i] = w[BQ // 2:]
            c11, c12, c21, c22 = _out4(ms)
            y = _join(c11, c21, c12, c22)
            if m == 0:
                vt_s[i] = _pk(y)
                for r in range(0, D, 8):
                    vmax = jnp.maximum(vmax, jnp.abs(y[r:r + 8]))
            else:
                q = _pk(y * (LOG2E * DH ** -0.5))
                for h in range(H):
                    e = h % G
                    qt_s[i * G + e, h // G, e * 8:e * 8 + 8, :] = q[h * 8:h * 8 + 8]
        lax.fori_loop(i + 1, jnp.minimum(i + 2, NB), lambda n, _: project_k(n), None)
        return vmax

    vmax = lax.fori_loop(0, NB, project, jnp.zeros((8, BQ), F32))
    cp_w1.start()
    cp_w2.start()

    def attend(u, carry):
        j, e = u // G, u % G
        zero = jnp.full((8, 128), j // NB, I32)
        lanes = [jnp.full((8, 128), e * DH, I32) + d for d in range(DH)]

        def load_q(h):
            qf = _unpk(qt_s[u, h, _ds(e, 8), :]).astype(F32)
            q = _unpk(qt_s[u, h] | jnp.full((G * 8, BQ), j // NB, I32))
            return q, [jnp.broadcast_to(qf[d:d + 1], (8, BQ)) for d in range(DH)]

        order = [(c, g) for c in range(NC) for g in range(6, -1, -1)]
        nm = len(order)
        tiles = [(h, c, h * nm + 7 * (c + 1) + LAG) for h in range(HP) for c in range(NC)]
        cuts = {t[2] for t in tiles} | {h * nm for h in range(HP + 1)} | {LAG}
        cuts = sorted(n for n in cuts if n <= HP * nm)
        p16, sums = {}, {}
        l = o = None
        nxt = load_q(0)
        for i0, i1 in zip(cuts, cuts[1:]):
            h, n0 = divmod(i0, nm)
            if n0 == 0:
                q, q_rows = nxt
                nxt = load_q(h + 1) if h + 1 < HP else None
                l = None if l is None else jnp.minimum(l, 0.0)
            groups = order[n0:n0 + i1 - i0]
            k = _unpk(jnp.concatenate(
                [k_s[h, (c * 8 + g) * 8:(c * 8 + g + 1) * 8, :] for c, g in groups], axis=0))
            p = jnp.exp2(_dot(k[:, :G * DH], q))
            for n, (c, g) in enumerate(groups):
                p16[h, c, g] = p[16 * n:16 * n + 16]
                l = _add_rows(l, p16[h, c, g])
                if g == 0:
                    kw = kw_s[h, c // 4, c % 4 * 8:c % 4 * 8 + 8, :]
                    p16[h, c, 7] = jnp.exp2(_vpu_scores(kw, lanes, q_rows))
                    l = _add_rows(l, p16[h, c, 7])
                    if nxt is not None:
                        z = zero
                        for m in range(0, BQ, 128):
                            z = z & pltpu.bitcast(nxt[1][c][:, m:m + 128], I32)
                        ls = [l[:, m:m + 128] for m in range(0, BQ, 128)]
                        ls[c % 4] = pltpu.bitcast(pltpu.bitcast(ls[c % 4], I32) | z, F32)
                        l = jnp.concatenate(ls, axis=1)
            sums[h] = l
            while tiles and (tiles[0][2] <= i1 or i1 == cuts[-1]):
                h, c, _ = tiles.pop(0)
                v = vt_s[c // 4, _ds(h * G + e, 8), c % 4 * CK:(c % 4 + 1) * CK]
                pv = _dot(_unpk(v), jnp.concatenate([p16.pop((h, c, g)) for g in range(8)], axis=0))
                if c == 0 and o is not None:
                    o = jnp.minimum(jnp.abs(o), 0.0)
                o = pv if o is None else o + pv
                if c == NC - 1:
                    ot_s[j, _ds(h * G + e, DH), :] = o
                    l_s[j, h * G + e] = sums[h]
        return carry

    lax.fori_loop(0, NB * G, attend, 0)

    def attend_with_max(n, carry):
        j, h = n // H, n % H
        q = _unpk(qt_s[j * G + h % G, h // G])

        def keys(c, state):
            m, l, o = state
            s = _dot(_unpk(k_s[h // G, _ds(c, BQ // 2), :])[:, :G * DH], q)
            m_new = jnp.maximum(m, jnp.max(s, axis=0, keepdims=True))
            a = jnp.exp2(m - m_new)
            p = jnp.exp2(s - m_new)
            pv = _dot(_unpk(vt_s[c, _ds(h, 8), :]), p.astype(BF16))
            return m_new, _add_rows(a * l, p), a * o + pv

        _, l, o = lax.fori_loop(0, NB, keys, (
            jnp.full((1, BQ), -np.inf, F32), jnp.zeros((8, BQ), F32), jnp.zeros((DH, BQ), F32)))
        ot_s[j, _ds(h, DH), :] = o
        l_s[j, h] = l
        return carry

    cp_w1.wait()
    cp_w2.wait()

    def finish(j, bounds):
        zero = jnp.full((8, 128), j // NB, I32)
        bounds = list(bounds)
        acts, heads, acc = {}, [], [None] * 7

        def product(a, b):
            r = _dot(a.astype(BF16), b.astype(BF16))
            h = len(heads)
            if h < H:
                z = jnp.concatenate([_after(r[:8, :128], zero)] * (BQ // 128), axis=1)
                l = jnp.sum(l_s[j, h] + z, axis=0, keepdims=True)
                bounds[:] = jnp.minimum(bounds[0], l), jnp.maximum(bounds[1], l)
                inv = pltpu.reciprocal(l, approx=True)
                heads.append(ot_s[j, h * DH:(h + 1) * DH, :] * (inv * (2.0 - l * inv)))
            return r

        def up(c):
            c0, c1 = FFN_COLS[c]
            w7 = _rhs7(*[w1_v[r:r + D // 2, n + c0:n + c1].astype(F32)
                         for r in (0, D // 2) for n in (0, F // 2)])
            h4 = _out4({n: product(_unpk(xs_s[j, n]), w7[n]) for n in ORDER})
            bias = [jnp.concatenate([b1_s[:, n + c0:n + c1]] * (BQ // 16), axis=0)
                    for n in (0, F // 2)]
            acts[c] = [_mish(h4[n] + bias[n % 2]) for n in range(4)]

        def down(a4, w4, order):
            a7, w7 = _lhs7(*a4), _rhs7(*w4)
            for n in order:
                m = product(a7[n], w7[n])
                if acc[n] is None and n >= 3:
                    x4 = _quads(x_blk(j)[...].astype(F32))
                    m = m + {3: x4[2], 4: x4[1], 5: x4[3], 6: x4[0] + x4[1] - x4[2]}[n]
                acc[n] = m if acc[n] is None else acc[n] + m

        def down_ffn(c, order=DOWN_ORDER):
            c0, c1 = FFN_COLS[c]
            down(acts.pop(c), [w2_v[r + c0:r + c1, n:n + D // 2].astype(F32)
                               for r in (0, F // 2) for n in (0, D // 2)], order)

        up(0)
        up(1)
        up(2)
        down_ffn(0)
        up(3)
        down_ffn(1)
        down_ffn(2)
        o = jnp.concatenate(
            [jnp.concatenate(heads[g:g + 8], axis=0).T for g in range(0, H, 8)], axis=1)
        down(_quads(o), _quads(x_blk(NB)[...].astype(F32)), DOWN_ORDER)
        down_ffn(3, ORDER)
        o_v[j] = _join(*_out4(acc)).astype(BF16)
        cp_o(j).start()
        return tuple(bounds)

    def attempt(state):
        @pl.when(state[0] == 1)
        def _():
            lax.fori_loop(0, NB * H, attend_with_max, 0)

        lo, hi = lax.fori_loop(
            0, NB, finish, (jnp.ones((1, BQ), F32), jnp.max(vmax, axis=0, keepdims=True)))
        safe = jnp.logical_and(lo >= 2.0 ** -30, hi <= 2.0 ** 56)
        for j in range(NB):
            cp_o(j).wait()
        return state[0] + 1, jnp.sum(jnp.where(safe, 0.0, 1.0))

    lax.while_loop(
        lambda s: jnp.logical_or(s[0] == 0, jnp.logical_and(s[0] == 1, s[1] > 0.0)),
        attempt, (0, 0.0))


@jax.jit
def pallas_parallel_sum__mha_block__dense_activation_mish__prompt_kernel(
    A_x: jax.Array,
    A_wqkv: jax.Array,
    A_wo: jax.Array,
    B_x: jax.Array,
    B_w1: jax.Array,
    B_b1: jax.Array,
    B_w2: jax.Array,
):
    del B_x
    hbm = pl.BlockSpec(memory_space=pl.ANY)
    out = pl.pallas_call(
        _kernel,
        out_shape=jax.ShapeDtypeStruct((S, D), BF16),
        in_specs=[hbm, hbm, hbm, hbm, pl.BlockSpec(memory_space=pltpu.VMEM), hbm],
        out_specs=hbm,
        scratch_shapes=[
            pltpu.VMEM((S + D, D), BF16),
            pltpu.VMEM((3, D, D), BF16),
            pltpu.VMEM((D, F), BF16),
            pltpu.VMEM((F, D), BF16),
            pltpu.VMEM((NB, BQ, D), BF16),
            pltpu.VMEM((2, 7, D // 4, D // 2), I32),
            pltpu.VMEM((8, F), F32),
            pltpu.VMEM((NB + 1, 7, BQ // 4, D // 2), I32),
            pltpu.VMEM((BQ // 2 + 32, D), I32),
            pltpu.VMEM((HP, S // 2, 128), I32),
            pltpu.VMEM((HP, NB, 32, 128), I32),
            pltpu.VMEM((NB * G, HP, G * 8, BQ), I32),
            pltpu.VMEM((NB, D // 2, BQ), I32),
            pltpu.VMEM((NB, D, BQ), F32),
            pltpu.VMEM((NB, H, 8, BQ), F32),
            pltpu.SemaphoreType.DMA((14,)),
        ],
        compiler_params=pltpu.CompilerParams(vmem_limit_bytes=100 << 20),
    )(A_x.reshape(S, D), A_wqkv, A_wo, B_w1, B_b1, B_w2)
    return out.reshape(1, S, D)
```

```python
import jax
import jax.numpy as jnp
import numpy as np
from jax import lax
import jax.experimental.pallas as pl
import jax.experimental.pallas.tpu as pltpu

F32, BF16, I32 = jnp.float32, jnp.bfloat16, jnp.int32
S, D, H, DH, F = 2048, 512, 32, 16, 1792
BQ = 512
NB = S // BQ
CK = 128
NC = S // CK
G = 2
HP = H // G
LAG = 9
LOG2E = 1.4426950408889634
ORDER = (1, 3, 2, 4, 0, 5, 6)
DOWN_ORDER = (3, 1, 2, 5, 0, 4, 6)
FFN_COLS = ((0, 256), (256, 512), (512, 768), (768, 896))


def _dot(a, b):
    return lax.dot_general(a, b, (((1,), (0,)), ((), ())), preferred_element_type=F32)


def _pk(x):
    return pltpu.bitcast(x.astype(BF16), I32)


def _unpk(x):
    return pltpu.bitcast(x, BF16)


def _after(x, zero):
    return pltpu.bitcast(pltpu.bitcast(x, I32) & zero, F32)


def _mish(h):
    e = jnp.exp2(jnp.minimum(h, 20.0) * LOG2E)
    n = e * (e + 2.0)
    return h * (n * pltpu.reciprocal(n + 2.0, approx=True))


def _pack2(hi, lo):
    lo = lax.shift_right_logical(pltpu.bitcast(lo.astype(BF16).astype(F32), I32), 16)
    hi = pltpu.bitcast(hi, I32)
    mag = jnp.maximum((hi & 0x7FFFFFFF) - lo + 0x8000, 0) & ~0xFFFF
    return (hi & ~0x7FFFFFFF) | mag | lo


def _vpu_scores(kw, lanes, q_rows):
    s = []
    for d in range(DH):
        w = jnp.take_along_axis(kw, lanes[d], axis=1, mode="promise_in_bounds")
        k = jnp.concatenate([pltpu.bitcast(w, F32), pltpu.bitcast(w << 16, F32)], axis=0)
        t = jnp.concatenate([k] * (BQ // 128), axis=1) * jnp.concatenate([q_rows[d]] * 2, axis=0)
        s.append(t if d < 2 else s[d - 2] + t)
    return s[-2] + s[-1]


def _add_rows(acc, p):
    for r in range(0, p.shape[0], 8):
        acc = p[r:r + 8] if acc is None else acc + p[r:r + 8]
    return acc


def _quads(x):
    m, n = x.shape[0] // 2, x.shape[1] // 2
    return x[:m, :n], x[:m, n:], x[m:, :n], x[m:, n:]


def _join(c11, c12, c21, c22):
    return jnp.concatenate(
        [jnp.concatenate([c11, c12], axis=1), jnp.concatenate([c21, c22], axis=1)], axis=0)


def _lhs7(a11, a12, a21, a22):
    return a11 + a22, a21 + a22, a11, a22, a11 + a12, a21 - a11, a12 - a22


def _rhs7(b11, b12, b21, b22):
    return b11 + b22, b11, b12 - b22, b21 - b11, b22, b11 + b12, b21 + b22


def _out4(m):
    return (((m[3] - m[4]) + m[0]) + m[6], m[2] + m[4],
            m[1] + m[3], ((m[2] - m[1]) + m[0]) + m[5])


def _ds(i, n):
    return pl.ds(pl.multiple_of(i * n, n), n)


def _kernel(x_hbm, wqkv_hbm, wo_hbm, w1_hbm, b1_hbm, w2_hbm, o_hbm,
            x_v, wqkv_v, w1_v, b1_v, w2_v, o_v, w_s, b1_s, xs_s, kc_s,
            k_s, kw_s, qt_s, vt_s, ot_s, l_s, sems):
    def x_blk(i):
        return x_v.at[_ds(i, BQ)]

    cp_x = [pltpu.make_async_copy(x_hbm.at[pl.ds(i * BQ, BQ)], x_blk(i), sems.at[i])
            for i in range(NB)]
    cp_x.append(pltpu.make_async_copy(wo_hbm, x_blk(NB), sems.at[NB]))
    cp_wq, cp_wk, cp_wv = [
        pltpu.make_async_copy(wqkv_hbm.at[:, pl.ds(i * D, D)], wqkv_v.at[i], sems.at[5 + i])
        for i in range(3)]
    cp_w1 = pltpu.make_async_copy(w1_hbm, w1_v, sems.at[8])
    cp_b1 = pltpu.make_async_copy(b1_hbm, b1_v, sems.at[14])
    cp_w2 = pltpu.make_async_copy(w2_hbm, w2_v, sems.at[9])

    def cp_o(j):
        return pltpu.make_async_copy(o_v.at[j], o_hbm.at[_ds(j, BQ)], sems.at[10 + j])

    def layernorm(i, r0=0, n=BQ // 2, after=None):
        quads = []
        for half in range(2):
            rows = pl.ds(pl.multiple_of(i * BQ + half * (BQ // 2) + r0, 16), n)
            x = x_v[rows, :].astype(F32)
            if after is not None:
                first = x[:, :128] + jnp.concatenate([after] * (n // 8), axis=0)
                x = jnp.concatenate([first, x[:, 128:]], axis=1)
            xc = x - jnp.mean(x, axis=-1, keepdims=True)
            xn = xc * lax.rsqrt(jnp.mean(xc * xc, axis=-1, keepdims=True) + 1e-5)
            quads += [xn[:, :D // 2], xn[:, D // 2:]]

        def store():
            for m, a in enumerate(_lhs7(*quads)):
                xs_s[i, m, r0 // 2:(r0 + n) // 2, :] = _pk(a)
        return store

    def project_k(i, first=False):
        if first:
            w7 = [w.astype(BF16) for w in _rhs7(*_quads(wqkv_v[1].astype(F32)))]
            for n in range(7):
                w_s[0, n] = pltpu.bitcast(w7[n], I32)
        else:
            w7 = [_unpk(w_s[0, n]) for n in range(7)]
        k = _join(*_out4({n: _dot(_unpk(xs_s[i, n]), w7[n]) for n in ORDER}))
        kc_s[:BQ // 2] = _pk(k)
        kc_s[BQ // 2:] = jnp.concatenate(
            [_pack2(k[e - 16:e - 8], k[e - 8:e]) for e in range(CK, BQ + 1, CK)], axis=0)

    def project(i, vmax, more=True):
        if more:
            pltpu.make_async_copy(x_blk(i + 1), x_blk(i + 1), sems.at[i + 1]).wait()
            zero = jnp.full((8, 128), i // NB, I32)
        for h in range(H):
            for e in range(G):
                if e != h % G:
                    qt_s[i * G + h % G, h // G, e * 8:e * 8 + 8, :] = jnp.zeros((8, BQ), I32)
        pieces = (16, 16, 16, 16, 32, 32, 32, 32, 32, 16, 16) if more else ()
        stores = {}
        for m, w7 in enumerate(([_unpk(w_s[1, n]) for n in range(7)],
                                _rhs7(*_quads(wqkv_v[0].astype(F32))))):
            ms = {}
            for t, n in enumerate(ORDER, 7 * m):
                ms[n] = _dot(_unpk(xs_s[i, n]), w7[n].astype(BF16))
                if t < len(pieces):
                    stores[t + 3] = layernorm(
                        i + 1, sum(pieces[:t]), pieces[t], _after(ms[n][:8, :128], zero))
                if t in stores:
                    stores.pop(t)()
                for h in range(HP):
                    if t == h * 13 // HP:
                        g, r = divmod(h * G * DH, 128)
                        k = kc_s[:, g * 128:(g + 1) * 128]
                        k = pltpu.roll(k, 128 - r, 1) if r else k
                        k_s[h, _ds(i, BQ // 2), :] = k[:BQ // 2]
                        kw_s[h, i] = k[BQ // 2:]
            y4 = _out4(ms)
            if m == 0:
                for y in y4:
                    for r in range(0, BQ // 2, 8):
                        vmax = jnp.maximum(vmax, jnp.abs(y[r:r + 8]))
            else:
                y4 = [y * (LOG2E * DH ** -0.5) for y in y4]
            t4 = {n: pltpu.bitcast(y4[n].astype(BF16).T, I32) for n in (2, 1, 3, 0)}
            y = _join(t4[0], t4[2], t4[1], t4[3])
            if m == 0:
                vt_s[i] = y
            else:
                for h in range(H):
                    e = h % G
                    qt_s[i * G + e, h // G, e * 8:e * 8 + 8, :] = y[h * 8:h * 8 + 8]
        if more:
            project_k(i + 1)
        return vmax

    cp_x[0].start()
    cp_wk.start()
    cp_x[0].wait()
    cp_wv.start()
    cp_wq.start()
    layernorm(0)()
    cp_wk.wait()
    for cp in cp_x[1:]:
        cp.start()
    project_k(0, first=True)
    cp_wv.wait()
    for n, w in enumerate(_rhs7(*_quads(wqkv_v[2].astype(F32)))):
        w_s[1, n] = _pk(w)
    cp_wq.wait()
    vmax = lax.fori_loop(0, NB - 1, project, jnp.zeros((8, D // 2), F32))
    vmax = project(NB - 1, vmax, more=False)
    vmax = jnp.concatenate([vmax, vmax], axis=1)
    cp_w1.start()
    cp_b1.start()
    cp_w2.start()

    def attend(u, carry):
        j, e = u // G, u % G
        zero = jnp.full((8, 128), j // NB, I32)
        lanes = [jnp.full((8, 128), e * DH, I32) + d for d in range(DH)]

        def load_q(h):
            qf = _unpk(qt_s[u, h, _ds(e, 8), :]).astype(F32)
            q = _unpk(qt_s[u, h] | jnp.full((G * 8, BQ), j // NB, I32))
            return q, [jnp.broadcast_to(qf[d:d + 1], (8, BQ)) for d in range(DH)]

        order = [(c, g) for c in range(NC) for g in range(6, -1, -1)]
        nm = len(order)
        tiles = [(h, c, h * nm + 7 * (c + 1) + LAG) for h in range(HP) for c in range(NC)]
        cuts = {t[2] for t in tiles} | {h * nm for h in range(HP + 1)} | {LAG}
        cuts = sorted(n for n in cuts if n <= HP * nm)
        p16, sums = {}, {}
        l = o = None
        nxt = load_q(0)
        for i0, i1 in zip(cuts, cuts[1:]):
            h, n0 = divmod(i0, nm)
            if n0 == 0:
                q, q_rows = nxt
                nxt = load_q(h + 1) if h + 1 < HP else None
                l = None if l is None else jnp.minimum(l, 0.0)
            groups = order[n0:n0 + i1 - i0]
            k = _unpk(jnp.concatenate(
                [k_s[h, (c * 8 + g) * 8:(c * 8 + g + 1) * 8, :] for c, g in groups], axis=0))
            p = jnp.exp2(_dot(k[:, :G * DH], q))
            for n, (c, g) in enumerate(groups):
                p16[h, c, g] = p[16 * n:16 * n + 16]
                l = _add_rows(l, p16[h, c, g])
                if g == 0:
                    kw = kw_s[h, c // 4, c % 4 * 8:c % 4 * 8 + 8, :]
                    p16[h, c, 7] = jnp.exp2(_vpu_scores(kw, lanes, q_rows))
                    l = _add_rows(l, p16[h, c, 7])
                    if nxt is not None:
                        z = zero
                        for m in range(128, BQ, 256):
                            z = z & pltpu.bitcast(nxt[1][c][:, m:m + 128], I32)
                        ls = [l[:, m:m + 128] for m in range(0, BQ, 128)]
                        ls[c % 4] = pltpu.bitcast(pltpu.bitcast(ls[c % 4], I32) | z, F32)
                        l = jnp.concatenate(ls, axis=1)
            sums[h] = l
            while tiles and (tiles[0][2] <= i1 or i1 == cuts[-1]):
                h, c, _ = tiles.pop(0)
                v = vt_s[c // 4, h * 16:h * 16 + 16, c % 4 * CK:(c % 4 + 1) * CK]
                v = jnp.where(lanes[0] == 0, v[:8], v[8:])
                pv = _dot(_unpk(v), jnp.concatenate([p16.pop((h, c, g)) for g in range(8)], axis=0))
                if c == 0 and o is not None:
                    o = _after(o, jnp.full((DH, BQ), j // NB, I32))
                o = pv if o is None else o + pv
                if c == NC - 1:
                    ot_s[j, _ds(h * G + e, DH), :] = o
                    l_s[j, h * G + e] = sums[h]
        return carry

    lax.fori_loop(0, NB * G, attend, 0)

    def attend_with_max(n, carry):
        j, h = n // H, n % H
        q = _unpk(qt_s[j * G + h % G, h // G])

        def keys(c, state):
            m, l, o = state
            s = _dot(_unpk(k_s[h // G, _ds(c, BQ // 2), :])[:, :G * DH], q)
            m_new = jnp.maximum(m, jnp.max(s, axis=0, keepdims=True))
            a = jnp.exp2(m - m_new)
            p = jnp.exp2(s - m_new)
            pv = _dot(_unpk(vt_s[c, _ds(h, 8), :]), p.astype(BF16))
            return m_new, _add_rows(a * l, p), a * o + pv

        _, l, o = lax.fori_loop(0, NB, keys, (
            jnp.full((1, BQ), -np.inf, F32), jnp.zeros((8, BQ), F32), jnp.zeros((DH, BQ), F32)))
        ot_s[j, _ds(h, DH), :] = o
        l_s[j, h] = l
        return carry

    cp_x[NB].wait()
    cp_w1.wait()
    cp_b1.wait()
    cp_w2.wait()
    b1_s[...] = jnp.broadcast_to(b1_v[...].astype(F32).reshape(1, F), (8, F))

    def finish(j, bounds):
        zero = jnp.full((8, 128), j // NB, I32)
        bounds = list(bounds)
        acts, heads, acc = {}, [], [None] * 7

        def product(a, b):
            r = _dot(a.astype(BF16), b.astype(BF16))
            h = len(heads)
            if h < H:
                z = jnp.concatenate([_after(r[:8, :128], zero)] * (BQ // 128), axis=1)
                l = jnp.sum(l_s[j, h] + z, axis=0, keepdims=True)
                bounds[:] = jnp.minimum(bounds[0], l), bounds[1] + l
                inv = pltpu.reciprocal(l, approx=True)
                heads.append(ot_s[j, h * DH:(h + 1) * DH, :] * (inv * (2.0 - l * inv)))
            return r

        def up(c):
            c0, c1 = FFN_COLS[c]
            w7 = _rhs7(*[w1_v[r:r + D // 2, n + c0:n + c1].astype(F32)
                         for r in (0, D // 2) for n in (0, F // 2)])
            ms = {}
            for n in ORDER:
                if ms:
                    yield
                ms[n] = product(_unpk(xs_s[j, n]), w7[n])
            h4 = _out4(ms)
            bias = [jnp.concatenate([b1_s[:, n + c0:n + c1]] * (BQ // 16), axis=0)
                    for n in (0, F // 2)]
            acts[c] = [_mish(h4[n] + bias[n % 2]) for n in range(4)]
            yield

        def down(a4, w4, order):
            a7, w7 = _lhs7(*a4), _rhs7(*w4)
            for n in order:
                m = product(a7[n], w7[n])
                if order is ORDER and n >= 3:
                    x4 = _quads(x_blk(j)[...].astype(F32))
                    m = m + {3: x4[2], 4: x4[1], 5: x4[3], 6: x4[0] + x4[1] - x4[2]}[n]
                acc[n] = m if acc[n] is None else acc[n] + m
                yield

        def down_ffn(c, order=DOWN_ORDER):
            c0, c1 = FFN_COLS[c]
            w4 = [w2_v[r + c0:r + c1, n:n + D // 2].astype(F32)
                  for r in (0, F // 2) for n in (0, D // 2)]
            yield from down(acts.pop(c), w4, order)

        def down_attention():
            o = jnp.concatenate(
                [jnp.concatenate(heads[g:g + 8], axis=0).T for g in range(0, H, 8)], axis=1)
            yield from down(_quads(o), _quads(x_blk(NB)[...].astype(F32)), DOWN_ORDER)

        for stage in ((up(0),), (up(1),), (up(2), down_ffn(0)), (up(3), down_ffn(1)),
                      (down_ffn(2), down_attention()), (down_ffn(3, ORDER),)):
            for _ in range(7):
                for step in stage:
                    next(step)
        o_v[j] = _join(*_out4(acc)).astype(BF16)
        cp_o(j).start()
        return tuple(bounds)

    def attempt(state):
        @pl.when(state[0] == 1)
        def _():
            lax.fori_loop(0, NB * H, attend_with_max, 0)

        v_bound = jnp.max(vmax, axis=0, keepdims=True) * 2.0 ** 74
        lo, hi = lax.fori_loop(0, NB, finish, (jnp.ones((1, BQ), F32), v_bound))
        safe = jnp.logical_and(lo >= 2.0 ** -30, hi <= 2.0 ** 100)
        for j in range(NB):
            cp_o(j).wait()
        return state[0] + 1, jnp.sum(jnp.where(safe, 0.0, 1.0))

    lax.while_loop(
        lambda s: jnp.logical_or(s[0] == 0, jnp.logical_and(s[0] == 1, s[1] > 0.0)),
        attempt, (0, 0.0))


@jax.jit
def pallas_parallel_sum__mha_block__dense_activation_mish__prompt_kernel(
    A_x: jax.Array,
    A_wqkv: jax.Array,
    A_wo: jax.Array,
    B_x: jax.Array,
    B_w1: jax.Array,
    B_b1: jax.Array,
    B_w2: jax.Array,
):
    del B_x
    hbm = pl.BlockSpec(memory_space=pl.ANY)
    out = pl.pallas_call(
        _kernel,
        out_shape=jax.ShapeDtypeStruct((S, D), BF16),
        in_specs=[hbm] * 6,
        out_specs=hbm,
        scratch_shapes=[
            pltpu.VMEM((S + D, D), BF16),
            pltpu.VMEM((3, D, D), BF16),
            pltpu.VMEM((D, F), BF16),
            pltpu.VMEM((F,), BF16),
            pltpu.VMEM((F, D), BF16),
            pltpu.VMEM((NB, BQ, D), BF16),
            pltpu.VMEM((2, 7, D // 4, D // 2), I32),
            pltpu.VMEM((8, F), F32),
            pltpu.VMEM((NB, 7, BQ // 4, D // 2), I32),
            pltpu.VMEM((BQ // 2 + 32, D), I32),
            pltpu.VMEM((HP, S // 2, 128), I32),
            pltpu.VMEM((HP, NB, 32, 128), I32),
            pltpu.VMEM((NB * G, HP, G * 8, BQ), I32),
            pltpu.VMEM((NB, D // 2, BQ), I32),
            pltpu.VMEM((NB, D, BQ), F32),
            pltpu.VMEM((NB, H, 8, BQ), F32),
            pltpu.SemaphoreType.DMA((15,)),
        ],
        compiler_params=pltpu.CompilerParams(vmem_limit_bytes=100 << 20),
    )(A_x.reshape(S, D), A_wqkv, A_wo, B_w1, B_b1, B_w2)
    return out.reshape(1, S, D)
```
